```python
import os as _os
_os.environ.setdefault("JAX_PLATFORMS", "cpu")
import jax
import jax.numpy as jnp

def _softmax(x, axis=-1):
    return jax.nn.softmax(x, axis=axis)
def _gelu(x):
    return jax.nn.gelu(x, approximate=True)
def _silu(x):
    return jax.nn.silu(x)
def _sigmoid(x):
    return jax.nn.sigmoid(x)
def _layernorm(x, axis=-1, eps=1e-5):
    m = jnp.mean(x, axis=axis, keepdims=True)
    v = jnp.var(x, axis=axis, keepdims=True)
    return (x - m) / jnp.sqrt(v + eps)
def _scatter_add(tgt, idx, src, axis=0):
    return tgt.at[idx].add(src)
def _segment_sum(src, seg, n):
    return jax.ops.segment_sum(src, seg, n)
class _Rng:
    def __init__(self, key):
        self._k = key
    def _next(self):
        self._k, sub = jax.random.split(self._k)
        return sub
    def normal(self, shape):
        return jax.random.normal(self._next(), shape, dtype=jnp.bfloat16)
    def randint(self, lo, hi, shape):
        return jax.random.randint(self._next(), shape, lo, hi, dtype=jnp.int32)
    def uniform(self, shape, lo=0.0, hi=1.0):
        return jax.random.uniform(self._next(), shape, jnp.bfloat16, lo, hi)
    def permutation(self, n):
        return jax.random.permutation(self._next(), n)


kernel_name = 'standalone__dense_activation_silu__prompt'

def setup_inputs():
    _rng = _Rng(jax.random.key(int.from_bytes(__import__("os").urandom(4), "little")))
    _w = (lambda a: (lambda t: t.astype(jnp.bfloat16) if jnp.issubdtype(t.dtype, jnp.floating) else t)(jnp.asarray(a)))
    B, S, D, F = 1, 2048, 448, 1792
    return {
        "x": _w((lambda *s: _rng.normal(s) * 0.05)(B, S, D)),
        "w1": _w((lambda *s: _rng.normal(s) * 0.05)(D, F) * (D ** -0.5)),
        "w2": _w((lambda *s: _rng.normal(s) * 0.05)(F, D) * (F ** -0.5)),
    }

def reference(x, w1, w2):
    h = jnp.einsum("bsd,df->bsf", x, w1)
    h = _silu(h)
    out = jnp.einsum("bsf,fd->bsd", h, w2)
    return out
```

```python
import jax
import jax.numpy as jnp
import jax.experimental.pallas as pl
import jax.experimental.pallas.tpu as pltpu


def _silu(h):
    d = 1.0 + jnp.exp(jnp.minimum(-h, 80.0))
    r = pl.reciprocal(d, approx=True)
    r = r + r * (1.0 - d * r)
    return h * r


@jax.jit
def pallas_standalone__dense_activation_silu__prompt_kernel(
    x: jax.Array,
    w1: jax.Array,
    w2: jax.Array,
):
    B, S, D = x.shape
    F = w1.shape[1]
    T = B * S
    ts, fc0, tail = 512, (128, 384, 1280), (384, 128)
    nt = T // ts
    ch0 = [(sum(fc0[:i]), fc0[i]) for i in range(len(fc0))]
    tl = [(T - ts + sum(tail[:i]), tail[i]) for i in range(len(tail))]
    assert sum(fc0) == F and sum(tail) == ts and T % ts == 0 and nt >= 2

    xT = jnp.swapaxes(x.reshape(T, D), 0, 1)
    w2T = jnp.swapaxes(w2, 0, 1)

    def kernel(x_hbm, w1_hbm, w2_hbm, o_hbm, x_v, w1_v, w2_v, w1t_v, o_v,
               sx, s1, s2, so, st, fence):
        def cp_x(i):
            a, n = (0, ts) if i == 0 else (ts, T - ts)
            return pltpu.make_async_copy(x_hbm.at[:, pl.ds(a, n)], x_v.at[:, pl.ds(a, n)], sx.at[i])

        def cp_w1(j):
            a, n = ch0[j]
            return pltpu.make_async_copy(w1_hbm.at[:, pl.ds(a, n)], w1_v.at[:, pl.ds(a, n)], s1.at[j])

        def cp_w2():
            return pltpu.make_async_copy(w2_hbm, w2_v, s2.at[0])

        def cp_o(i):
            return pltpu.make_async_copy(o_v.at[:, pl.ds(i * ts, ts)], o_hbm.at[:, pl.ds(i * ts, ts)], so.at[i])

        def cp_t(i):
            a, n = tl[i]
            return pltpu.make_async_copy(o_v.at[:, pl.ds(a, n)], o_hbm.at[:, pl.ds(a, n)], st.at[i])

        def in_order():
            pl.semaphore_signal(fence.at[0], 1)
            pl.semaphore_wait(fence.at[0], 1)

        cp_x(0).start()
        for j in range(len(ch0)):
            in_order()
            cp_w1(j).start()
        in_order()
        cp_w2().start()
        in_order()
        cp_x(1).start()

        def up(a, n, xt):
            h = jnp.dot(w1t_v[pl.ds(a, n), :], xt, preferred_element_type=jnp.float32)
            return _silu(h).astype(jnp.bfloat16)

        def down(act):
            return jnp.dot(w2_v[...], act, preferred_element_type=jnp.float32).astype(o_v.dtype)

        cp_x(0).wait()
        x0 = x_v[:, pl.ds(0, ts)]
        acts = []
        for j, (a, n) in enumerate(ch0):
            cp_w1(j).wait()
            w1t_v[pl.ds(a, n), :] = w1_v[:, pl.ds(a, n)].T
            acts.append(up(a, n, x0))
        cp_w2().wait()
        cp_x(1).wait()
        o_v[:, pl.ds(0, ts)] = down(jnp.concatenate(acts, axis=0))
        cp_o(0).start()

        for i in range(1, nt - 1):
            o_v[:, pl.ds(i * ts, ts)] = down(up(0, F, x_v[:, pl.ds(i * ts, ts)]))
            cp_o(i).start()

        act = up(0, F, x_v[:, pl.ds(T - ts, ts)])
        for i, (a, n) in enumerate(tl):
            lo = a - (T - ts)
            o_v[:, pl.ds(a, n)] = down(act[:, lo:lo + n])
            cp_t(i).start()

        for i in range(nt - 1):
            cp_o(i).wait()
        for i in range(len(tl)):
            cp_t(i).wait()

    any_spec = pl.BlockSpec(memory_space=pl.ANY)
    oT = pl.pallas_call(
        kernel,
        in_specs=[any_spec, any_spec, any_spec],
        out_specs=any_spec,
        out_shape=jax.ShapeDtypeStruct((D, T), x.dtype),
        scratch_shapes=[
            pltpu.VMEM((D, T), x.dtype),
            pltpu.VMEM((D, F), w1.dtype),
            pltpu.VMEM((D, F), w2.dtype),
            pltpu.VMEM((F, D), w1.dtype),
            pltpu.VMEM((D, T), x.dtype),
            pltpu.SemaphoreType.DMA((2,)),
            pltpu.SemaphoreType.DMA((len(ch0),)),
            pltpu.SemaphoreType.DMA((1,)),
            pltpu.SemaphoreType.DMA((nt,)),
            pltpu.SemaphoreType.DMA((len(tl),)),
            pltpu.SemaphoreType.REGULAR((1,)),
        ],
        compiler_params=pltpu.CompilerParams(vmem_limit_bytes=100 * 1024 * 1024),
    )(xT, w1, w2T)
    return jnp.swapaxes(oT, 0, 1).reshape(B, S, D)
```

```python
import jax
import jax.numpy as jnp
from jax import lax
import jax.experimental.pallas as pl
import jax.experimental.pallas.tpu as pltpu

_LOG2E = 1.4426950408889634
_F32_MAX = 3.4028234663852886e38
_NT = (((1,), (1,)), ((), ()))


def _silu(h):
    d = 1.0 + jnp.exp2(h * (-_LOG2E))
    r = pl.reciprocal(d, approx=True)
    return (h * r) * (2.0 - jnp.minimum(d, _F32_MAX) * r)


@jax.jit
def pallas_standalone__dense_activation_silu__prompt_kernel(
    x: jax.Array,
    w1: jax.Array,
    w2: jax.Array,
):
    B, S, D = x.shape
    F = w1.shape[1]
    T = B * S
    KM = D // 128 * 128
    T0, C0 = 512, 512
    UP = 256
    HEAD = 512
    outs = [(0, 512, 0, D), (512, 512, 0, D), (1024, 512, 0, D), (1536, 256, 0, D),
            (1792, 256, 0, KM), (1792, 256, KM, D - KM)]
    assert (T, D, F) == (2048, 448, 1792)

    xT = jnp.swapaxes(x.reshape(T, D), 0, 1)
    w2T = jnp.swapaxes(w2, 0, 1)

    def kernel(x_hbm, w1_hbm, w2_hbm, o_hbm, x_v, w1_v, w2_v, o_v, p_v, in_sem, out_sem, fence):
        def load(i, src, dst, r0, r1, c0, c1):
            idx = (pl.ds(r0, r1 - r0), pl.ds(c0, c1 - c0))
            return pltpu.make_async_copy(src.at[idx], dst.at[idx], in_sem.at[i])

        x_slab0 = load(0, x_hbm, x_v, KM, D, 0, T0)
        w_slab0 = load(1, w1_hbm, w1_v, KM, D, 0, C0)
        w_slab1 = load(2, w1_hbm, w1_v, KM, D, C0, F)
        x_slab1 = load(3, x_hbm, x_v, KM, D, T0, T)
        w1_main = load(4, w1_hbm, w1_v, 0, KM, 0, F)
        x_main = load(5, x_hbm, x_v, 0, KM, 0, T)
        w2_all = load(6, w2_hbm, w2_v, 0, D, 0, F)
        stores = [
            pltpu.make_async_copy(o_v.at[pl.ds(r, m), pl.ds(a, n)],
                                  o_hbm.at[pl.ds(r, m), pl.ds(a, n)], out_sem.at[i])
            for i, (a, n, r, m) in enumerate(outs)
        ]

        for i, cp in enumerate((x_slab0, w_slab0, w_slab1, x_slab1, w1_main, x_main, w2_all)):
            if i:
                pl.semaphore_signal(fence.at[0], 1)
                pl.semaphore_wait(fence.at[0], 1)
            cp.start()

        def slab_tokens(a, b):
            return x_v[pl.ds(KM, D - KM), pl.ds(a, b - a)].T

        def slab(a, b, xt, f0, f1):
            p_v[pl.ds(a, b - a), pl.ds(f0, f1 - f0)] = jnp.dot(
                xt, w1_v[pl.ds(KM, D - KM), pl.ds(f0, f1 - f0)], preferred_element_type=jnp.float32)

        acts = {}

        def up(a):
            h = jnp.dot(x_v[pl.ds(0, KM), pl.ds(a, UP)].T, w1_v[pl.ds(0, KM), :],
                        preferred_element_type=jnp.float32)
            acts[a] = _silu(h + p_v[pl.ds(a, UP), :]).astype(jnp.bfloat16)

        def down(i):
            a, n, r, m = outs[i]
            act = jnp.concatenate([acts[t] for t in range(a, a + n, UP)], axis=0)
            o = lax.dot_general(w2_v[pl.ds(r, m), :], act, _NT, preferred_element_type=jnp.float32)
            o_v[pl.ds(r, m), pl.ds(a, n)] = o.astype(o_v.dtype)
            stores[i].start()

        x_slab0.wait()
        xt0 = slab_tokens(0, T0)
        w_slab0.wait()
        slab(0, T0, xt0, 0, C0)

        w_slab1.wait()
        x_slab1.wait()
        slab(0, T0, xt0, C0, F)
        for a in range(T0, T, 512):
            slab(a, a + 512, slab_tokens(a, a + 512), 0, F)

        w1_main.wait()
        x_main.wait()
        for a in range(0, HEAD, UP):
            up(a)

        w2_all.wait()
        for i, (a, n, _, _) in enumerate(outs):
            for t in range(a, a + n, UP):
                if t not in acts:
                    up(t)
            down(i)

        for cp in stores:
            cp.wait()

    any_spec = pl.BlockSpec(memory_space=pl.ANY)
    oT = pl.pallas_call(
        kernel,
        in_specs=[any_spec, any_spec, any_spec],
        out_specs=any_spec,
        out_shape=jax.ShapeDtypeStruct((D, T), x.dtype),
        scratch_shapes=[
            pltpu.VMEM((D, T), x.dtype),
            pltpu.VMEM((D, F), w1.dtype),
            pltpu.VMEM((D, F), w2.dtype),
            pltpu.VMEM((D, T), x.dtype),
            pltpu.VMEM((T, F), jnp.float32),
            pltpu.SemaphoreType.DMA((7,)),
            pltpu.SemaphoreType.DMA((len(outs),)),
            pltpu.SemaphoreType.REGULAR((1,)),
        ],
        compiler_params=pltpu.CompilerParams(vmem_limit_bytes=100 * 1024 * 1024),
    )(xT, w1, w2T)
    return jnp.swapaxes(oT, 0, 1).reshape(B, S, D)
```

```python
import jax
import jax.numpy as jnp
from jax import lax
import jax.experimental.pallas as pl
import jax.experimental.pallas.tpu as pltpu

_LOG2E = 1.4426950408889634
_F32_MAX = 3.4028234663852886e38
_NT = (((1,), (1,)), ((), ()))
_FLAGS = {"XLA_TPU_RESCHEDULE_DMA_DONES": True} if jax.__version_info__ >= (0, 12) else None


def _silu(h):
    d = 1.0 + jnp.exp2(h * (-_LOG2E))
    r = pl.reciprocal(d, approx=True)
    return (h * r) * (2.0 - jnp.minimum(d, _F32_MAX) * r)


@jax.jit
def pallas_standalone__dense_activation_silu__prompt_kernel(
    x: jax.Array,
    w1: jax.Array,
    w2: jax.Array,
):
    B, S, D = x.shape
    F = w1.shape[1]
    T = B * S
    assert (T, D, F) == (2048, 448, 1792)
    KM = D // 128 * 128
    T0, C0 = 512, 512
    UP = 256
    HEAD = 512
    outs = [(0, 512, 0, D), (512, 512, 0, D), (1024, 512, 0, D), (1536, 256, 0, D),
            (1792, 256, 0, KM), (1792, 256, KM, D - KM)]

    xT = jnp.swapaxes(x.reshape(T, D), 0, 1)
    w2T = jnp.swapaxes(w2, 0, 1)

    def kernel(x_hbm, w1_hbm, w2_hbm, o_hbm, x_v, w1_v, w2_v, o_v, p_v, in_sem, out_sem, fence):
        def load(i, src, dst, r0, r1, c0, c1):
            idx = (pl.ds(r0, r1 - r0), pl.ds(c0, c1 - c0))
            return pltpu.make_async_copy(src.at[idx], dst.at[idx], in_sem.at[i])

        x_slab0 = load(0, x_hbm, x_v, KM, D, 0, T0)
        w_slab0 = load(1, w1_hbm, w1_v, KM, D, 0, C0)
        w_slab1 = load(2, w1_hbm, w1_v, KM, D, C0, F)
        x_slab1 = load(3, x_hbm, x_v, KM, D, T0, T)
        w1_main = load(4, w1_hbm, w1_v, 0, KM, 0, F)
        x_main = load(5, x_hbm, x_v, 0, KM, 0, T)
        w2_all = load(6, w2_hbm, w2_v, 0, D, 0, F)
        stores = [
            pltpu.make_async_copy(o_v.at[pl.ds(r, m), pl.ds(a, n)],
                                  o_hbm.at[pl.ds(r, m), pl.ds(a, n)], out_sem.at[i])
            for i, (a, n, r, m) in enumerate(outs)
        ]

        for i, cp in enumerate((x_slab0, w_slab0, w_slab1, x_slab1, w1_main, x_main, w2_all)):
            if i:
                pl.semaphore_signal(fence.at[0], 1)
                pl.semaphore_wait(fence.at[0], 1)
            cp.start()

        def not_before(buf, val, row, col):
            buf[pl.ds(D, 16), pl.ds(0, 128)] = val[row:row + 16, col:col + 128].astype(buf.dtype)

        def slab_tokens(a, n):
            return x_v[pl.ds(KM, D - KM), pl.ds(a, n)].T

        def slab(a, xt, f0, f1):
            p = jnp.dot(xt, w1_v[pl.ds(KM, D - KM), pl.ds(f0, f1 - f0)],
                        preferred_element_type=jnp.float32)
            p_v[pl.ds(a, xt.shape[0]), pl.ds(f0, f1 - f0)] = p
            return p

        acts = {}

        def up(a):
            h = jnp.dot(x_v[pl.ds(0, KM), pl.ds(a, UP)].T, w1_v[pl.ds(0, KM), :],
                        preferred_element_type=jnp.float32)
            acts[a] = _silu(h + p_v[pl.ds(a, UP), :]).astype(jnp.bfloat16)
            return h

        def down(i):
            a, n, r, m = outs[i]
            act = jnp.concatenate([acts[t] for t in range(a, a + n, UP)], axis=0)
            o = lax.dot_general(w2_v[pl.ds(r, m), :], act, _NT, preferred_element_type=jnp.float32)
            o_v[pl.ds(r, m), pl.ds(a, n)] = o.astype(o_v.dtype)
            stores[i].start()

        x_slab0.wait()
        w_slab0.wait()
        xt0 = slab_tokens(0, T0)
        p = slab(0, xt0, 0, C0)

        not_before(w1_v, p, 256, 0)
        w_slab1.wait()
        p = slab(0, xt0, C0, F)

        not_before(x_v, p, 256, 512)
        x_slab1.wait()
        for a in range(T0, T, 512):
            p = slab(a, slab_tokens(a, 512), 0, F)

        not_before(w1_v, p, 400, 1024)
        w1_main.wait()
        x_main.wait()
        for a in range(0, HEAD, UP):
            h = up(a)

        not_before(w2_v, h, 0, 0)
        w2_all.wait()
        for i, (a, n, _, _) in enumerate(outs):
            for t in range(a, a + n, UP):
                if t not in acts:
                    up(t)
            down(i)

        for cp in stores:
            cp.wait()

    any_spec = pl.BlockSpec(memory_space=pl.ANY)
    oT = pl.pallas_call(
        kernel,
        in_specs=[any_spec, any_spec, any_spec],
        out_specs=any_spec,
        out_shape=jax.ShapeDtypeStruct((D, T), x.dtype),
        scratch_shapes=[
            pltpu.VMEM((D + 16, T), x.dtype),
            pltpu.VMEM((D + 16, F), w1.dtype),
            pltpu.VMEM((D + 16, F), w2.dtype),
            pltpu.VMEM((D, T), x.dtype),
            pltpu.VMEM((T, F), jnp.float32),
            pltpu.SemaphoreType.DMA((7,)),
            pltpu.SemaphoreType.DMA((len(outs),)),
            pltpu.SemaphoreType.REGULAR((1,)),
        ],
        compiler_params=pltpu.CompilerParams(vmem_limit_bytes=64 * 1024 * 1024, flags=_FLAGS),
    )(xT, w1, w2T)
    return jnp.swapaxes(oT, 0, 1).reshape(B, S, D)
```

```python
import jax
import jax.numpy as jnp
from jax import lax
import jax.experimental.pallas as pl
import jax.experimental.pallas.tpu as pltpu

_LOG2E = 1.4426950408889634
_F32_MAX = 3.4028234663852886e38
_NT = (((1,), (1,)), ((), ()))
_FLAGS = {"XLA_TPU_RESCHEDULE_DMA_DONES": True} if jax.__version_info__ >= (0, 12) else None


def _silu(h):
    d = 1.0 + jnp.exp2(h * (-_LOG2E))
    r = pl.reciprocal(d, approx=True)
    return (h * r) * (2.0 - jnp.minimum(d, _F32_MAX) * r)


@jax.jit
def pallas_standalone__dense_activation_silu__prompt_kernel(
    x: jax.Array,
    w1: jax.Array,
    w2: jax.Array,
):
    B, S, D = x.shape
    F = w1.shape[1]
    T = B * S
    assert (T, D, F) == (2048, 448, 1792)
    KM = D // 128 * 128
    T0, C0 = 512, 512
    UP = 256
    HEAD = 1024
    outs = [(0, 1024, 0, D), (1024, 768, 0, D), (1792, 256, 0, KM), (1792, 256, KM, D - KM)]

    xT = jnp.swapaxes(x.reshape(T, D), 0, 1)
    w2T = jnp.swapaxes(w2, 0, 1)

    def kernel(x_hbm, w1_hbm, w2_hbm, o_hbm, x_v, w1_v, w2_v, o_v, p_v, in_sem, out_sem, fence):
        def load(i, src, dst, r0, r1, c0, c1):
            idx = (pl.ds(r0, r1 - r0), pl.ds(c0, c1 - c0))
            return pltpu.make_async_copy(src.at[idx], dst.at[idx], in_sem.at[i])

        x_slab0 = load(0, x_hbm, x_v, KM, D, 0, T0)
        w_slab0 = load(1, w1_hbm, w1_v, KM, D, 0, C0)
        w_slab1 = load(2, w1_hbm, w1_v, KM, D, C0, F)
        x_slab1 = load(3, x_hbm, x_v, KM, D, T0, T)
        w1_main = load(4, w1_hbm, w1_v, 0, KM, 0, F)
        x_main = load(5, x_hbm, x_v, 0, KM, 0, T)
        w2_all = load(6, w2_hbm, w2_v, 0, D, 0, F)
        stores = [
            pltpu.make_async_copy(o_v.at[pl.ds(r, m), pl.ds(a, n)],
                                  o_hbm.at[pl.ds(r, m), pl.ds(a, n)], out_sem.at[i])
            for i, (a, n, r, m) in enumerate(outs)
        ]

        for i, cp in enumerate((x_slab0, w_slab0, w_slab1, x_slab1, w1_main, x_main, w2_all)):
            if i:
                pl.semaphore_signal(fence.at[0], 1)
                pl.semaphore_wait(fence.at[0], 1)
            cp.start()

        def not_before(buf, tile):
            buf[pl.ds(D, 16), pl.ds(0, tile.shape[1])] = tile.astype(buf.dtype)

        def slab_tokens(a):
            return x_v[pl.ds(KM, D - KM), pl.ds(a, UP)].T

        def slab(a, xt, f0, f1):
            p = jnp.dot(xt, w1_v[pl.ds(KM, D - KM), pl.ds(f0, f1 - f0)],
                        preferred_element_type=jnp.float32)
            p_v[pl.ds(a, UP), pl.ds(f0, f1 - f0)] = p
            return p

        acts = {}

        def up(a):
            h = jnp.dot(x_v[pl.ds(0, KM), pl.ds(a, UP)].T, w1_v[pl.ds(0, KM), :],
                        preferred_element_type=jnp.float32)
            acts[a] = _silu(h + p_v[pl.ds(a, UP), :]).astype(jnp.bfloat16)
            return h

        def down(i):
            a, n, r, m = outs[i]
            act = jnp.concatenate([acts[t] for t in range(a, a + n, UP)], axis=0)
            o = lax.dot_general(w2_v[pl.ds(r, m), :], act, _NT, preferred_element_type=jnp.float32)
            o_v[pl.ds(r, m), pl.ds(a, n)] = o.astype(o_v.dtype)
            stores[i].start()

        x_slab0.wait()
        first = [(a, slab_tokens(a)) for a in range(0, T0, UP)]
        not_before(w1_v, first[0][1][:16])
        w_slab0.wait()
        for a, xt in first:
            p = slab(a, xt, 0, C0)

        not_before(w1_v, p[:16, :128])
        w_slab1.wait()
        for a, xt in first:
            p = slab(a, xt, C0, F)

        not_before(x_v, p[:16, :128])
        x_slab1.wait()
        for a in range(T0, T, UP):
            p = slab(a, slab_tokens(a), 0, F)

        not_before(w1_v, p[128:144, 512:640])
        w1_main.wait()
        x_main.wait()
        hs = [up(a) for a in range(0, HEAD, UP)]

        not_before(w2_v, hs[2][:16, :128])
        w2_all.wait()
        for i, (a, n, _, _) in enumerate(outs):
            for t in range(a, a + n, UP):
                if t not in acts:
                    up(t)
            down(i)

        for cp in stores:
            cp.wait()

    any_spec = pl.BlockSpec(memory_space=pl.ANY)
    oT = pl.pallas_call(
        kernel,
        in_specs=[any_spec, any_spec, any_spec],
        out_specs=any_spec,
        out_shape=jax.ShapeDtypeStruct((D, T), x.dtype),
        scratch_shapes=[
            pltpu.VMEM((D + 16, T), x.dtype),
            pltpu.VMEM((D + 16, F), w1.dtype),
            pltpu.VMEM((D + 16, F), w2.dtype),
            pltpu.VMEM((D, T), x.dtype),
            pltpu.VMEM((T, F), jnp.float32),
            pltpu.SemaphoreType.DMA((7,)),
            pltpu.SemaphoreType.DMA((len(outs),)),
            pltpu.SemaphoreType.REGULAR((1,)),
        ],
        compiler_params=pltpu.CompilerParams(vmem_limit_bytes=64 * 1024 * 1024, flags=_FLAGS),
    )(xT, w1, w2T)
    return jnp.swapaxes(oT, 0, 1).reshape(B, S, D)
```

```python
import jax
import jax.numpy as jnp
from jax import lax
import jax.experimental.pallas as pl
import jax.experimental.pallas.tpu as pltpu

_LOG2E = 1.4426950408889634
_F32_MAX = 3.4028234663852886e38
_NT = (((1,), (1,)), ((), ()))
_FLAGS = {"XLA_TPU_RESCHEDULE_DMA_DONES": True} if jax.__version_info__ >= (0, 12) else None


def _silu(h):
    d = 1.0 + jnp.exp2(h * (-_LOG2E))
    r = pl.reciprocal(d, approx=True)
    return (h * r) * (2.0 - jnp.minimum(d, _F32_MAX) * r)


@jax.jit
def pallas_standalone__dense_activation_silu__prompt_kernel(
    x: jax.Array,
    w1: jax.Array,
    w2: jax.Array,
):
    B, S, D = x.shape
    F = w1.shape[1]
    T = B * S
    assert (T, D, F) == (2048, 448, 1792)
    KM = D // 128 * 128
    T0, C0 = 512, 512
    UP = 256
    HEAD = 1024
    outs = [(0, 1024, 0, D), (1024, 768, 0, D), (1792, 256, 0, KM), (1792, 256, KM, D - KM)]

    xT = jnp.swapaxes(x.reshape(T, D), 0, 1)
    w2T = jnp.swapaxes(w2, 0, 1)

    def kernel(x_hbm, w1_hbm, w2_hbm, o_hbm, x_v, w1_v, w2_v, o_v, p_v, sems):
        def load(sem, src, dst, r0, r1, c0, c1):
            idx = (pl.ds(r0, r1 - r0), pl.ds(c0, c1 - c0))
            return pltpu.make_async_copy(src.at[idx], dst.at[idx], sems.at[sem])

        x_slab0 = load(0, x_hbm, x_v, KM, D, 0, T0)
        w_slab0 = load(1, w1_hbm, w1_v, KM, D, 0, C0)
        w_slab1 = load(2, w1_hbm, w1_v, KM, D, C0, F)
        x_slab1 = load(0, x_hbm, x_v, KM, D, T0, T)
        w1_main = load(1, w1_hbm, w1_v, 0, KM, 0, F)
        x_main = load(1, x_hbm, x_v, 0, KM, 0, T)
        w2_all = load(2, w2_hbm, w2_v, 0, D, 0, F)
        stores = [
            pltpu.make_async_copy(o_v.at[pl.ds(r, m), pl.ds(a, n)],
                                  o_hbm.at[pl.ds(r, m), pl.ds(a, n)], sems.at[0])
            for a, n, r, m in outs
        ]

        def start_in_order(fence):
            for i, cp in enumerate((x_slab0, w_slab0, w_slab1)):
                if i:
                    pl.semaphore_signal(fence, 1)
                    pl.semaphore_wait(fence, 1)
                cp.start()

        def not_before(buf, tile):
            buf[pl.ds(D, 16), pl.ds(0, tile.shape[1])] = tile.astype(buf.dtype)

        def slab_tokens(a):
            return x_v[pl.ds(KM, D - KM), pl.ds(a, UP)].T

        def slab(a, xt, f0, f1):
            p = jnp.dot(xt, w1_v[pl.ds(KM, D - KM), pl.ds(f0, f1 - f0)],
                        preferred_element_type=jnp.float32)
            p_v[pl.ds(a, UP), pl.ds(f0, f1 - f0)] = p
            return p

        acts = {}

        def up(a):
            h = jnp.dot(x_v[pl.ds(0, KM), pl.ds(a, UP)].T, w1_v[pl.ds(0, KM), :],
                        preferred_element_type=jnp.float32)
            acts[a] = _silu(h + p_v[pl.ds(a, UP), :]).astype(jnp.bfloat16)
            return h

        def down(a, n, r, m):
            act = jnp.concatenate([acts[t] for t in range(a, a + n, UP)], axis=0)
            o = lax.dot_general(w2_v[pl.ds(r, m), :], act, _NT, preferred_element_type=jnp.float32)
            o_v[pl.ds(r, m), pl.ds(a, n)] = o.astype(o_v.dtype)

        pl.run_scoped(start_in_order, pltpu.SemaphoreType.REGULAR(()))

        x_slab0.wait()
        x_slab1.start()
        first = [(a, slab_tokens(a)) for a in range(0, T0, UP)]
        not_before(w1_v, first[0][1][:16])
        w_slab0.wait()
        w1_main.start()
        x_main.start()
        for a, xt in first:
            p = slab(a, xt, 0, C0)

        not_before(w1_v, p[:16, :128])
        w_slab1.wait()
        w2_all.start()
        for a, xt in first:
            p = slab(a, xt, C0, F)

        not_before(x_v, p[:16, :128])
        x_slab1.wait()
        for a in range(T0, T, UP):
            p = slab(a, slab_tokens(a), 0, F)

        not_before(w1_v, p[128:144, 512:640])
        w1_main.wait()
        x_main.wait()
        hs = [up(a) for a in range(0, HEAD, UP)]

        not_before(w2_v, hs[2][:16, :128])
        w2_all.wait()
        for (a, n, r, m), store in zip(outs, stores):
            for t in range(a, a + n, UP):
                if t not in acts:
                    up(t)
            down(a, n, r, m)
            store.start()

        for store in stores:
            store.wait()

    any_spec = pl.BlockSpec(memory_space=pl.ANY)
    oT = pl.pallas_call(
        kernel,
        in_specs=[any_spec, any_spec, any_spec],
        out_specs=any_spec,
        out_shape=jax.ShapeDtypeStruct((D, T), x.dtype),
        scratch_shapes=[
            pltpu.VMEM((D + 16, T), x.dtype),
            pltpu.VMEM((D + 16, F), w1.dtype),
            pltpu.VMEM((D + 16, F), w2.dtype),
            pltpu.VMEM((D, T), x.dtype),
            pltpu.VMEM((T, F), jnp.float32),
            pltpu.SemaphoreType.DMA((3,)),
        ],
        compiler_params=pltpu.CompilerParams(vmem_limit_bytes=64 * 1024 * 1024, flags=_FLAGS),
    )(xT, w1, w2T)
    return jnp.swapaxes(oT, 0, 1).reshape(B, S, D)
```
